```python
import os as _os
_os.environ.setdefault("JAX_PLATFORMS", "cpu")
import jax
import jax.numpy as jnp

def _softmax(x, axis=-1):
    return jax.nn.softmax(x, axis=axis)
def _gelu(x):
    return jax.nn.gelu(x, approximate=True)
def _silu(x):
    return jax.nn.silu(x)
def _sigmoid(x):
    return jax.nn.sigmoid(x)
def _layernorm(x, axis=-1, eps=1e-5):
    m = jnp.mean(x, axis=axis, keepdims=True)
    v = jnp.var(x, axis=axis, keepdims=True)
    return (x - m) / jnp.sqrt(v + eps)
def _scatter_add(tgt, idx, src, axis=0):
    return tgt.at[idx].add(src)
def _segment_sum(src, seg, n):
    return jax.ops.segment_sum(src, seg, n)
class _Rng:
    def __init__(self, key):
        self._k = key
    def _next(self):
        self._k, sub = jax.random.split(self._k)
        return sub
    def normal(self, shape):
        return jax.random.normal(self._next(), shape, dtype=jnp.bfloat16)
    def randint(self, lo, hi, shape):
        return jax.random.randint(self._next(), shape, lo, hi, dtype=jnp.int32)
    def uniform(self, shape, lo=0.0, hi=1.0):
        return jax.random.uniform(self._next(), shape, jnp.bfloat16, lo, hi)
    def permutation(self, n):
        return jax.random.permutation(self._next(), n)


kernel_name = 'standalone__dense_activation_gelu__prompt'

def setup_inputs():
    _rng = _Rng(jax.random.key(int.from_bytes(__import__("os").urandom(4), "little")))
    _w = (lambda a: (lambda t: t.astype(jnp.bfloat16) if jnp.issubdtype(t.dtype, jnp.floating) else t)(jnp.asarray(a)))
    B, S, D, F = 1, 2048, 640, 1728
    return {
        "x": _w((lambda *s: _rng.normal(s) * 0.05)(B, S, D)),
        "w1": _w((lambda *s: _rng.normal(s) * 0.05)(D, F) * (D ** -0.5)),
        "b1": _w((lambda *s: _rng.normal(s) * 0.05)(F) * 0.01),
        "w2": _w((lambda *s: _rng.normal(s) * 0.05)(F, D) * (F ** -0.5)),
        "b2": _w((lambda *s: _rng.normal(s) * 0.05)(D) * 0.01),
    }

def reference(x, w1, b1, w2, b2):
    h = jnp.einsum("bsd,df->bsf", x, w1) + b1
    h = _gelu(h)
    return jnp.einsum("bsf,fd->bsd", h, w2) + b2
```

```python
import jax
import jax.numpy as jnp
import numpy as np
from jax import lax
from jax.experimental import pallas as pl
from jax.experimental.pallas import tpu as pltpu

_SQRT_2_OVER_PI = float(np.sqrt(2.0 / np.pi))
_NT = (((1,), (1,)), ((), ()))


def _gelu(h):
    return 0.5 * h * (1.0 + jnp.tanh(_SQRT_2_OVER_PI * (h + 0.044715 * (h * h * h))))


@jax.jit
def pallas_standalone__dense_activation_gelu__prompt_kernel(x, w1, b1, w2, b2):
    B, S, D = x.shape
    F = w1.shape[1]
    f32, bf16 = jnp.float32, x.dtype
    bm = 512
    nb = S // bm
    assert B == 1 and S % bm == 0

    dma = [('x', 0, 256), ('w1', 0, 256), ('x', 256, 256), ('w1', 256, 256), ('w1', 512, 512), ('w1', 1024, 704),
           ('w2', 0, 256), ('w2', 256, 256), ('w2', 512, 512), ('w2', 1024, 704)]
    phase0 = [(0, 256, 0, 256), (256, 256, 0, 256), (0, 512, 256, 256), (0, 512, 512, 512), (0, 512, 1024, 704)]
    base = dict(x=0, w1=S, w2=S + F)
    nd = len(dma)
    SX = nd + 2
    SO = SX + nb - 1
    slab = 128

    def kernel(x_h, w1_h, b1_h, w2_h, b2_h, o_h, buf, b1_v, b2_v, o_v, sem):
        src = dict(x=x_h, w1=w1_h, w2=w2_h)
        cps = [pltpu.make_async_copy(src[n].at[pl.ds(s, z)], buf.at[pl.ds(base[n] + s, z)], sem.at[i])
               for i, (n, s, z) in enumerate(dma)]
        cb = [pltpu.make_async_copy(b1_h, b1_v, sem.at[nd]), pltpu.make_async_copy(b2_h, b2_v, sem.at[nd + 1])]

        def xcopy(j):
            r = (j + 1) * bm
            if not isinstance(j, int):
                r = pl.multiple_of(r, bm)
            return pltpu.make_async_copy(x_h.at[pl.ds(r, bm)], buf.at[pl.ds(r, bm)], sem.at[SX + j])

        for c in cps[:2]:
            c.start()
        for c in cb:
            c.start()
        for c in cps[2:]:
            c.start()
        for j in range(nb - 1):
            xcopy(j).start()
        nxt = [0]

        def need(name, s, z):
            hi = max(i for i, (n, ds_, dz) in enumerate(dma) if n == name and ds_ < s + z and s < ds_ + dz)
            while nxt[0] <= hi:
                cps[nxt[0]].wait()
                nxt[0] += 1
                if nxt[0] == 2:
                    for c in cb:
                        c.wait()

        def finish(acc, ms, mz, sl):
            for c in range(0, D, sl):
                a = acc[:, c:c + sl] + b2_v[pl.ds(c, sl)].astype(f32).reshape(1, sl)
                o_v[pl.ds(ms, mz), pl.ds(c, sl)] = a.astype(o_v.dtype)
                pltpu.make_async_copy(o_v.at[pl.ds(ms, mz), pl.ds(c, sl)], o_h.at[pl.ds(ms, mz), pl.ds(c, sl)],
                                      sem.at[SO]).start()

        def mm1(ms, mz, fs, fz):
            xv = buf[pl.ds(ms, mz), :]
            wv = buf[pl.ds(base['w1'] + fs, fz), :]
            h = lax.dot_general(xv, wv, _NT, preferred_element_type=f32)
            h = h + b1_v[pl.ds(fs, fz)].astype(f32).reshape(1, fz)
            return _gelu(h).astype(bf16)

        pieces = {}
        for (r0, rz, fs, fz) in phase0:
            need('x', r0, rz)
            need('w1', fs, fz)
            pieces[(r0, rz, fs, fz)] = mm1(r0, rz, fs, fz)
        acc = None
        for (fs, fz) in sorted({(fs, fz) for (_, _, fs, fz) in pieces}):
            rows = sorted((k for k in pieces if k[2] == fs and k[3] == fz), key=lambda k: k[0])
            g = jnp.concatenate([pieces[k] for k in rows], axis=0) if len(rows) > 1 else pieces[rows[0]]
            need('w2', fs, fz)
            p = jnp.dot(g, buf[pl.ds(base['w2'] + fs, fz), :], preferred_element_type=f32)
            acc = p if acc is None else acc + p
        while nxt[0] < nd:
            cps[nxt[0]].wait()
            nxt[0] += 1
        finish(acc, 0, bm, D)

        def body(j, carry):
            ms = pl.multiple_of((j + 1) * bm, bm)
            xcopy(j).wait()
            g = mm1(ms, bm, 0, F)
            acc = jnp.dot(g, buf[pl.ds(base['w2'], F), :], preferred_element_type=f32)
            finish(acc, ms, bm, slab)
            return carry

        lax.fori_loop(0, nb - 1, body, 0)
        pltpu.make_async_copy(o_v, o_h, sem.at[SO]).wait()

    out = pl.pallas_call(
        kernel,
        in_specs=[pl.BlockSpec(memory_space=pltpu.HBM)] * 5,
        out_specs=pl.BlockSpec(memory_space=pltpu.HBM),
        out_shape=jax.ShapeDtypeStruct((S, D), x.dtype),
        scratch_shapes=[
            pltpu.VMEM((S + 2 * F, D), bf16), pltpu.VMEM((F,), bf16), pltpu.VMEM((D,), bf16), pltpu.VMEM((S, D), bf16),
            pltpu.SemaphoreType.DMA((SO + 1,)),
        ],
        compiler_params=pltpu.CompilerParams(vmem_limit_bytes=64 << 20,
                                             flags={'XLA_TPU_RESCHEDULE_DMA_DONES': True}),
    )(x.reshape(S, D), w1.T, b1, w2, b2)
    return out.reshape(B, S, D)
```

```python
import jax
import jax.numpy as jnp
import numpy as np
from jax import lax
from jax.experimental import pallas as pl
from jax.experimental.pallas import tpu as pltpu

_SQRT_2_OVER_PI = float(np.sqrt(2.0 / np.pi))
_NT = (((1,), (1,)), ((), ()))
_LANES = 128
_PAD = 16


def _gelu(h):
    return 0.5 * h * (1.0 + jnp.tanh(_SQRT_2_OVER_PI * (h + 0.044715 * (h * h * h))))


def _cat(xs, axis):
    return xs[0] if len(xs) == 1 else jnp.concatenate(xs, axis=axis)


@jax.jit
def pallas_standalone__dense_activation_gelu__prompt_kernel(x, w1, b1, w2, b2):
    B, S, D = x.shape
    F = w1.shape[1]
    f32, bf16 = jnp.float32, x.dtype
    BM = 512
    FM = F // _LANES * _LANES
    R = F - FM
    nb = S // BM
    assert B == 1 and S % BM == 0 and D == 5 * _LANES and FM == 13 * _LANES and R == 64

    n_chunks = [(0, 512), (512, 512), (1024, FM - 1024)]
    k_slices = [(0, 128), (128, 256), (384, D - 384)]
    loads = []
    for k0, kz in k_slices:
        loads.append(("x", 0, BM, k0, kz))
        loads += [("w1", f0, fz, k0, kz) for f0, fz in n_chunks]
    loads.append(("w1", FM, R, 0, D))
    loads += [("w2", 0, 1024, 0, D), ("w2", 1024, F - 1024, 0, D)]
    loads += [("x", j * BM, BM, 0, D) for j in range(1, nb)]
    nl = len(loads)
    bias_after = 2
    k_chunks0 = [(0, 256), (256, 256), (512, 512), (1024, F - 1024)]
    row0 = dict(x=0, w1=0, w2=F)
    SEM_OUT = nl + 2

    def kernel(x_h, w1t_h, b1_h, w2_h, b2_h, o_h, xbuf, wbuf, b1_v, b2_v, o_v, sem):
        src = dict(x=x_h, w1=w1t_h, w2=w2_h)
        copies = []
        for i, (n, r, rz, c, cz) in enumerate(loads):
            dst = xbuf if n == "x" else wbuf
            copies.append(pltpu.make_async_copy(
                src[n].at[pl.ds(r, rz), pl.ds(c, cz)],
                dst.at[pl.ds(row0[n] + r, rz), pl.ds(c, cz)], sem.at[i]))
        cb1 = pltpu.make_async_copy(b1_h, b1_v, sem.at[nl])
        cb2 = pltpu.make_async_copy(b2_h, b2_v, sem.at[nl + 1])
        order = copies[:bias_after] + [cb1, cb2] + copies[bias_after:]
        for c in order:
            c.start()
        waited = [0]

        def wait_through(last):
            hi = [i for i, o in enumerate(order) if o is last][0]
            while waited[0] <= hi:
                order[waited[0]].wait()
                waited[0] += 1

        def need(name, r, rz, c=0, cz=D):
            hit = [copies[i] for i, (n, lr, lz, lc, lcz) in enumerate(loads)
                   if n == name and lr < r + rz and r < lr + lz and lc < c + cz and c < lc + lcz]
            wait_through(hit[-1])

        def pin(name, value):
            tile = value[0:_PAD, 0:_LANES].astype(bf16)
            if name == "x":
                xbuf[pl.ds(S, _PAD), pl.ds(0, _LANES)] = tile
            else:
                wbuf[pl.ds(2 * F, _PAD), pl.ds(0, _LANES)] = tile

        def activation(h, f0, fz):
            wait_through(cb1)
            return _gelu(h + b1_v[pl.ds(f0, fz)].astype(f32).reshape(1, fz))

        def mm1(r, f0, fz, k0=0, kz=D):
            need("x", r, BM, k0, kz)
            need("w1", f0, fz, k0, kz)
            return lax.dot_general(xbuf[pl.ds(r, BM), pl.ds(k0, kz)],
                                   wbuf[pl.ds(f0, fz), pl.ds(k0, kz)], _NT, preferred_element_type=f32)

        def mm1_remainder(r):
            need("x", r, BM)
            need("w1", FM, R)
            ht = lax.dot_general(wbuf[pl.ds(FM, R), :], xbuf[pl.ds(r, BM), :], _NT,
                                 preferred_element_type=f32)
            return activation(ht.T, FM, R)

        def mm2(g, f0, fz):
            need("w2", f0, fz)
            return jnp.dot(g, wbuf[pl.ds(F + f0, fz), :], preferred_element_type=f32)

        def finish(acc, r, pieces):
            wait_through(cb2)
            for r0, rz, c, cz in pieces:
                a = acc[r0:r0 + rz, c:c + cz] + b2_v[pl.ds(c, cz)].astype(f32).reshape(1, cz)
                o_v[pl.ds(r + r0, rz), pl.ds(c, cz)] = a.astype(o_v.dtype)
                pltpu.make_async_copy(o_v.at[pl.ds(r + r0, rz), pl.ds(c, cz)],
                                      o_h.at[pl.ds(r + r0, rz), pl.ds(c, cz)], sem.at[SEM_OUT]).start()

        partial, act = {}, []
        steps = [(k0, kz, f0, fz) for k0, kz in k_slices for f0, fz in n_chunks]
        for i, (k0, kz, f0, fz) in enumerate(steps):
            p = mm1(0, f0, fz, k0, kz)
            partial[f0] = p if k0 == 0 else partial[f0] + p
            if k0 + kz == D:
                act.append(activation(partial[f0], f0, fz))
            if i + 1 < len(steps) and steps[i + 1][0] != k0:
                pin("x", p)
            pin("w", p)
        act.append(mm1_remainder(0))
        g0 = _cat(act, 1)
        acc = None
        for i, (f0, fz) in enumerate(k_chunks0):
            if i == len(k_chunks0) - 1:
                wait_through(order[-1])
            p = mm2(g0[:, f0:f0 + fz].astype(bf16), f0, fz)
            acc = p if acc is None else acc + p
        finish(acc, 0, [(0, BM, 0, D)])

        for j in range(1, nb):
            r = j * BM
            rem = mm1_remainder(r)
            main = activation(mm1(r, 0, FM), 0, FM)
            acc = mm2(_cat([main, rem], 1).astype(bf16), 0, F)
            if j < nb - 1:
                finish(acc, r, [(0, BM, 0, D)])
            else:
                finish(acc, r, [(r0, _LANES, c, _LANES)
                                for c in range(0, D, _LANES) for r0 in range(0, BM, _LANES)])
        pltpu.make_async_copy(o_v, o_h, sem.at[SEM_OUT]).wait()

    out = pl.pallas_call(
        kernel,
        in_specs=[pl.BlockSpec(memory_space=pltpu.HBM)] * 5,
        out_specs=pl.BlockSpec(memory_space=pltpu.HBM),
        out_shape=jax.ShapeDtypeStruct((S, D), x.dtype),
        scratch_shapes=[
            pltpu.VMEM((S + _PAD, D), bf16),
            pltpu.VMEM((2 * F + _PAD, D), bf16),
            pltpu.VMEM((F,), bf16),
            pltpu.VMEM((D,), bf16),
            pltpu.VMEM((S, D), bf16),
            pltpu.SemaphoreType.DMA((SEM_OUT + 1,)),
        ],
        compiler_params=pltpu.CompilerParams(
            vmem_limit_bytes=64 << 20,
            flags={"XLA_TPU_RESCHEDULE_DMA_DONES": True},
            disable_semaphore_checks=True,
        ),
    )(x.reshape(S, D), w1.T, b1, w2, b2)
    return out.reshape(B, S, D)
```

```python
import jax
import jax.numpy as jnp
import numpy as np
from jax import lax
from jax.experimental import pallas as pl
from jax.experimental.pallas import tpu as pltpu

_SQRT_2_OVER_PI = float(np.sqrt(2.0 / np.pi))
_NT = (((1,), (1,)), ((), ()))
_L = 128
_BM = 512
_PAD = 16


def _gelu(h):
    return 0.5 * h * (1.0 + jnp.tanh(_SQRT_2_OVER_PI * (h + 0.044715 * (h * h * h))))


def _cat(xs, axis):
    return xs[0] if len(xs) == 1 else jnp.concatenate(xs, axis=axis)


def _overlap(a, az, b, bz):
    return a < b + bz and b < a + az


@jax.jit
def pallas_standalone__dense_activation_gelu__prompt_kernel(x, w1, b1, w2, b2):
    B, S, D = x.shape
    F = w1.shape[1]
    f32, bf16 = jnp.float32, x.dtype
    FM = F // _L * _L
    R = F - FM
    nb = S // _BM
    assert (B, S, D, F) == (1, 2048, 640, 1728), "schedule below is laid out for these shapes"

    KA, KB = 256, D - 256
    loads = [
        ("x", 0, 256, 0, KA), ("w1", 0, 128, 0, KA), ("w1", 128, 128, 0, KA), "bias",
        ("w1", 256, 256, 0, KA), ("x", 256, 256, 0, KA),
        ("w1", 512, 256, 0, KA), ("w1", 768, 256, 0, KA), ("w1", 1024, 256, 0, KA),
        ("w1", 1280, 256, 0, KA), ("w1", 1536, 128, 0, KA),
        ("x", 0, _BM, KA, KB), ("w1", 0, 256, KA, KB), ("w1", FM, R, 0, D),
        ("w1", 256, 512, KA, KB), ("w1", 768, 896, KA, KB),
        ("w2", 0, 1024, 0, D), ("w2", 1024, F - 1024, 0, D),
    ] + [("x", j * _BM, _BM, 0, D) for j in range(1, nb)]
    chunks = [c for c in loads if c != "bias"]
    nc = len(chunks)
    SEM_OUT = nc + 2

    steps0 = [
        ("m", 0, 256, 0, 128, 0, KA), ("m", 0, 256, 128, 128, 0, KA), ("m", 0, 256, 256, 256, 0, KA),
        ("m", 256, 256, 0, 512, 0, KA),
        ("m", 0, _BM, 512, 256, 0, KA), ("m", 0, _BM, 768, 256, 0, KA), ("m", 0, _BM, 1024, 256, 0, KA),
        ("m", 0, _BM, 1280, 256, 0, KA), ("m", 0, _BM, 1536, 128, 0, KA),
        ("m", 0, _BM, 0, 256, KA, KB), ("t",), ("m", 0, _BM, 256, 512, KA, KB), ("m", 0, _BM, 768, 896, KA, KB),
    ]
    k_chunks0 = [(0, 512), (512, 512), (1024, F - 1024)]

    def steps_later(j):
        return [("m", 0, _BM, 0, j * _L, 0, D), ("t",), ("m", 0, _BM, j * _L, FM - j * _L, 0, D)]

    tail = [(r, _L, c, _L) for c in range(0, D - _L, _L) for r in range(0, _BM, _L)]
    tail += [(0, 128, D - _L, _L), (128, 128, D - _L, _L), (256, 128, D - _L, _L),
             (384, 64, D - _L, _L), (448, 32, D - _L, _L), (480, 32, D - _L, _L)]
    row0 = dict(x=0, w1=0, w2=F)

    def kernel(x_h, w1t_h, b1_h, w2_h, b2_h, o_h, xbuf, wbuf, b1_v, b2_v, o_v, sem):
        src = dict(x=x_h, w1=w1t_h, w2=w2_h)
        copies = [
            pltpu.make_async_copy(src[n].at[pl.ds(r, rz), pl.ds(c, cz)],
                                  (xbuf if n == "x" else wbuf).at[pl.ds(row0[n] + r, rz), pl.ds(c, cz)],
                                  sem.at[i])
            for i, (n, r, rz, c, cz) in enumerate(chunks)]
        cb1 = pltpu.make_async_copy(b1_h, b1_v, sem.at[nc])
        cb2 = pltpu.make_async_copy(b2_h, b2_v, sem.at[nc + 1])
        order, k = [], 0
        for c in loads:
            if c == "bias":
                order += [cb1, cb2]
            else:
                order.append(copies[k])
                k += 1
        for c in order:
            c.start()
        waited = [0]

        def position(c):
            return [i for i, o in enumerate(order) if o is c][0]

        def wait_through(hi):
            while waited[0] <= hi:
                order[waited[0]].wait()
                waited[0] += 1

        def last_needed(name, r, rz, c=0, cz=D):
            return max(position(copies[i]) for i, (n, lr, lz, lc, lcz) in enumerate(chunks)
                       if n == name and _overlap(r, rz, lr, lz) and _overlap(c, cz, lc, lcz))

        def pin(name, value):
            tile = value[0:_PAD, 0:_L].astype(bf16)
            if name == "x":
                xbuf[pl.ds(S, _PAD), pl.ds(0, _L)] = tile
            else:
                wbuf[pl.ds(2 * F, _PAD), pl.ds(0, _L)] = tile

        def activation(h, f0, fz):
            wait_through(position(cb1))
            return _gelu(h + b1_v[pl.ds(f0, fz)].astype(f32).reshape(1, fz))

        def finish(acc, r, pieces):
            wait_through(position(cb2))
            for r0, rz, c, cz in pieces:
                a = acc[r0:r0 + rz, c:c + cz] + b2_v[pl.ds(c, cz)].astype(f32).reshape(1, cz)
                o_v[pl.ds(r + r0, rz), pl.ds(c, cz)] = a.astype(o_v.dtype)
                pltpu.make_async_copy(o_v.at[pl.ds(r + r0, rz), pl.ds(c, cz)],
                                      o_h.at[pl.ds(r + r0, rz), pl.ds(c, cz)], sem.at[SEM_OUT]).start()

        def block(r, steps, k_chunks, pieces, first):
            done, partial = [], {}
            row_cuts = sorted({0, _BM} | {e for s in steps if s[0] == "m" for e in (s[1], s[1] + s[2])})
            col_cuts = sorted({e for s in steps if s[0] == "m" for e in (s[3], s[3] + s[4])})
            prev = None
            for s in steps:
                if s[0] == "m":
                    _, r0, rz, f0, fz, k0, kz = s
                    hi = max(last_needed("x", r + r0, rz, k0, kz), last_needed("w1", f0, fz, k0, kz))
                else:
                    hi = max(last_needed("x", r, _BM), last_needed("w1", FM, R))
                if hi >= waited[0] and prev is not None:
                    fresh = {"x" if any(o is copies[i] and chunks[i][0] == "x" for i in range(nc)) else "w"
                             for o in order[waited[0]:hi + 1] if o is not cb1 and o is not cb2}
                    for name in sorted(fresh):
                        pin(name, prev)
                wait_through(hi)
                if s[0] == "t":
                    ht = lax.dot_general(wbuf[pl.ds(FM, R), :], xbuf[pl.ds(r, _BM), :], _NT,
                                         preferred_element_type=f32)
                    done.append((0, _BM, FM, R, activation(ht.T, FM, R)))
                    prev = None
                    continue
                p = lax.dot_general(xbuf[pl.ds(r + r0, rz), pl.ds(k0, kz)],
                                    wbuf[pl.ds(f0, fz), pl.ds(k0, kz)], _NT, preferred_element_type=f32)
                prev = p
                if kz == D:
                    done.append((r0, rz, f0, fz, activation(p, f0, fz)))
                    continue
                rs = [e for e in row_cuts if r0 <= e <= r0 + rz]
                cs = [e for e in col_cuts if f0 <= e <= f0 + fz]
                complete, rows = True, []
                for ra, rb in zip(rs[:-1], rs[1:]):
                    row = []
                    for ca, cb in zip(cs[:-1], cs[1:]):
                        t = p[ra - r0:rb - r0, ca - f0:cb - f0]
                        seen, total = partial.get((ra, ca), (0, None))
                        total = t if total is None else total + t
                        partial[(ra, ca)] = (seen + kz, total)
                        complete = complete and seen + kz == D
                        row.append(total)
                    rows.append(row)
                if complete:
                    h = _cat([_cat(row, 1) for row in rows], 0)
                    done.append((r0, rz, f0, fz, activation(h, f0, fz)))

            def g(f0, fz):
                cuts = sorted({f0, f0 + fz} | {e for d in done for e in (d[2], d[2] + d[3]) if f0 < e < f0 + fz})
                cols = []
                for c0, c1 in zip(cuts[:-1], cuts[1:]):
                    rows = sorted((d for d in done if d[2] <= c0 and c1 <= d[2] + d[3]), key=lambda d: d[0])
                    cols.append(_cat([d[4][:, c0 - d[2]:c1 - d[2]] for d in rows], 0))
                return _cat(cols, 1).astype(bf16)

            acc = None
            for i, (f0, fz) in enumerate(k_chunks):
                if first and i == len(k_chunks) - 1:
                    wait_through(len(order) - 1)
                lhs = g(f0, fz)
                wait_through(last_needed("w2", f0, fz))
                p = jnp.dot(lhs, wbuf[pl.ds(F + f0, fz), :], preferred_element_type=f32)
                acc = p if acc is None else acc + p
            finish(acc, r, pieces)

        block(0, steps0, k_chunks0, [(0, _BM, 0, D)], first=True)
        for j in range(1, nb):
            block(j * _BM, steps_later(j), [(0, F)], tail if j == nb - 1 else [(0, _BM, 0, D)], first=False)
        pltpu.make_async_copy(o_v, o_h, sem.at[SEM_OUT]).wait()

    out = pl.pallas_call(
        kernel,
        in_specs=[pl.BlockSpec(memory_space=pltpu.HBM)] * 5,
        out_specs=pl.BlockSpec(memory_space=pltpu.HBM),
        out_shape=jax.ShapeDtypeStruct((S, D), x.dtype),
        scratch_shapes=[
            pltpu.VMEM((S + _PAD, D), bf16),
            pltpu.VMEM((2 * F + _PAD, D), bf16),
            pltpu.VMEM((F,), bf16),
            pltpu.VMEM((D,), bf16),
            pltpu.VMEM((S, D), bf16),
            pltpu.SemaphoreType.DMA((SEM_OUT + 1,)),
        ],
        compiler_params=pltpu.CompilerParams(
            vmem_limit_bytes=64 << 20,
            flags={"XLA_TPU_RESCHEDULE_DMA_DONES": True},
            disable_semaphore_checks=True,
        ),
    )(x.reshape(S, D), w1.T, b1, w2, b2)
    return out.reshape(B, S, D)
```
